```python
import os as _os
_os.environ.setdefault("JAX_PLATFORMS", "cpu")
import jax
import jax.numpy as jnp

def _softmax(x, axis=-1):
    return jax.nn.softmax(x, axis=axis)
def _gelu(x):
    return jax.nn.gelu(x, approximate=True)
def _silu(x):
    return jax.nn.silu(x)
def _sigmoid(x):
    return jax.nn.sigmoid(x)
def _layernorm(x, axis=-1, eps=1e-5):
    m = jnp.mean(x, axis=axis, keepdims=True)
    v = jnp.var(x, axis=axis, keepdims=True)
    return (x - m) / jnp.sqrt(v + eps)
def _scatter_add(tgt, idx, src, axis=0):
    return tgt.at[idx].add(src)
def _segment_sum(src, seg, n):
    return jax.ops.segment_sum(src, seg, n)
class _Rng:
    def __init__(self, key):
        self._k = key
    def _next(self):
        self._k, sub = jax.random.split(self._k)
        return sub
    def normal(self, shape):
        return jax.random.normal(self._next(), shape, dtype=jnp.bfloat16)
    def randint(self, lo, hi, shape):
        return jax.random.randint(self._next(), shape, lo, hi, dtype=jnp.int32)
    def uniform(self, shape, lo=0.0, hi=1.0):
        return jax.random.uniform(self._next(), shape, jnp.bfloat16, lo, hi)
    def permutation(self, n):
        return jax.random.permutation(self._next(), n)


kernel_name = 'parallel_sum__linear_kernel_hedgehog__dense_activation_gelu__prompt'

def setup_inputs():
    _rng = _Rng(jax.random.key(int.from_bytes(__import__("os").urandom(4), "little")))
    _w = (lambda a: (lambda t: t.astype(jnp.bfloat16) if jnp.issubdtype(t.dtype, jnp.floating) else t)(jnp.asarray(a)))
    def _A_setup():
        B, S, D, H = 1, 2048, 448, 16
        Dh = D // H
        return {
            "x": _w((lambda *s: _rng.normal(s) * 0.05)(B, S, D)),
            "wqkv": _w((lambda *s: _rng.normal(s) * 0.2)(D, 3 * D)),
            "w_phi": _w((lambda *s: _rng.normal(s) * 0.2)(H, Dh, Dh) * (Dh ** -0.5)),
            "wo": _w((lambda *s: _rng.normal(s) * 0.05)(D, D)),
        }
    _A_in = _A_setup()

    def _B_setup():
        B, S, D, F = 1, 2048, 448, 1792
        return {
            "x": _w((lambda *s: _rng.normal(s) * 0.05)(B, S, D)),
            "w1": _w((lambda *s: _rng.normal(s) * 0.2)(D, F) * (D ** -0.5)),
            "b1": _w((lambda *s: _rng.normal(s) * 0.2)(F) * 0.01),
            "w2": _w((lambda *s: _rng.normal(s) * 0.2)(F, D) * (F ** -0.5)),
            "b2": _w((lambda *s: _rng.normal(s) * 0.05)(D) * 0.01),
        }
    _B_in = _B_setup()

    return {
        "A_x": _A_in["x"],
        "A_wqkv": _A_in["wqkv"],
        "A_w_phi": _A_in["w_phi"],
        "A_wo": _A_in["wo"],
        "B_x": _B_in["x"],
        "B_w1": _B_in["w1"],
        "B_b1": _B_in["b1"],
        "B_w2": _B_in["w2"],
        "B_b2": _B_in["b2"],
    }

def reference(A_x, A_wqkv, A_w_phi, A_wo, B_x, B_w1, B_b1, B_w2, B_b2):
    def _A_ref(x, wqkv, w_phi, wo):
        B, S, D = x.shape
        H = 16; Dh = D // H
        qkv = (lambda x, *d: x.transpose(*d))((x @ wqkv).reshape(B, S, 3, H, Dh), 2, 0, 3, 1, 4)
        q, k, v = qkv[0], qkv[1], qkv[2]
        pq = jnp.einsum("bhsd,hdf->bhsf", q, w_phi)
        pk = jnp.einsum("bhsd,hdf->bhsf", k, w_phi)
        phi_q = jnp.concatenate([_softmax(pq, axis=-1), _softmax(-pq, axis=-1)], axis=-1)
        phi_k = jnp.concatenate([_softmax(pk, axis=-1), _softmax(-pk, axis=-1)], axis=-1)
        kv = jnp.einsum("bhsf,bhsd->bhfd", phi_k, v)
        z  = jnp.einsum("bhsf->bhf", phi_k)
        num = jnp.einsum("bhqf,bhfd->bhqd", phi_q, kv)
        den = jnp.einsum("bhqf,bhf->bhq", phi_q, z)[..., None] + 1e-6
        o = num / den
        return (lambda x, *d: x.transpose(*d))(o, 0, 2, 1, 3).reshape(B, S, D) @ wo

    def _B_ref(x, w1, b1, w2, b2):
        h = jnp.einsum("bsd,df->bsf", x, w1) + b1
        h = _gelu(h)
        return jnp.einsum("bsf,fd->bsd", h, w2) + b2

    x = A_x
    xn = _layernorm(x, axis=-1)
    return x + _A_ref(xn, A_wqkv, A_w_phi, A_wo) + _B_ref(xn, B_w1, B_b1, B_w2, B_b2)
```

```python
import jax
import jax.numpy as jnp
import jax.experimental.pallas as pl
import jax.experimental.pallas.tpu as pltpu

H = 16
G = 4
TS = 512
FC = 256

_NT = (((1,), (1,)), ((), ()))
_TN = (((0,), (0,)), ((), ()))
F32 = jnp.float32
BF16 = jnp.bfloat16


def _dot(a, b, dims=(((1,), (0,)), ((), ()))):
    return jax.lax.dot_general(a, b, dims, preferred_element_type=F32)


def _iota(shape, d):
    return jax.lax.broadcasted_iota(jnp.int32, shape, d)


def _fdiv(i, n):
    return jnp.floor((i.astype(F32) + 0.5) * (1.0 / n)).astype(jnp.int32)


def _features(p, Dh):
    T = p.shape[1]
    R = 4 * Dh
    n = R // 8
    outs = []
    for g in range(G):
        pg = p[g * R:(g + 1) * R].reshape(n, 8, T)
        mx = jnp.max(pg, axis=0)
        mn = jnp.min(pg, axis=0)
        mx = jnp.maximum(mx, pltpu.roll(mx, 4, 0))
        mn = jnp.minimum(mn, pltpu.roll(mn, 4, 0))
        e1 = jnp.exp(pg - mx[None])
        e2 = jnp.exp(mn[None] - pg)
        s1 = jnp.sum(e1, axis=0)
        s2 = jnp.sum(e2, axis=0)
        s1 = s1 + pltpu.roll(s1, 4, 0)
        s2 = s2 + pltpu.roll(s2, 4, 0)
        f1 = (e1 * (1.0 / s1)[None]).reshape(R, T).astype(BF16)
        f2 = (e2 * (1.0 / s2)[None]).reshape(R, T).astype(BF16)
        outs.append((f1, f2))
    return outs


def _kernel(x_ref, wqkv_ref, wphi_ref, b1_ref, b2_ref, wo_hbm, w1_hbm, w2_hbm,
            o_ref,
            w1_s, w2_s, wo_s, wqk_s, wv_s, wop_s, kv_s, kvt_s, phiq_s, acc_s, sems,
            *, D, F):
    ph = pl.program_id(0)
    t = pl.program_id(1)
    Dh = D // H
    R = 4 * Dh
    DP = H * 32

    cp1 = pltpu.make_async_copy(w1_hbm, w1_s, sems.at[0])
    cp2 = pltpu.make_async_copy(w2_hbm, w2_s, sems.at[1])
    cp3 = pltpu.make_async_copy(wo_hbm, wo_s, sems.at[2])

    @pl.when(jnp.logical_and(ph == 0, t == 0))
    def _():
        cp1.start()
        cp2.start()
        cp3.start()
        r = _iota((D, Dh), 0)
        g_r = _fdiv(r, R)
        f_r = (r - g_r * R) >> 2
        et = (f_r == _iota((D, Dh), 1)).astype(BF16)
        ct = _dot(et, wphi_ref[...], _NT)
        r = _iota((D, D), 0)
        head_r = _fdiv(r, R) * 4 + (r & 3)
        head_c = _fdiv(_iota((D, D), 1), Dh)
        bd = jnp.where(head_r == head_c, ct, 0.0).astype(BF16)
        wqk_s[0:D, :] = _dot(bd, wqkv_ref[:, 0:D], _NT).astype(BF16)
        wqk_s[D:2 * D, :] = _dot(bd, wqkv_ref[:, D:2 * D], _NT).astype(BF16)
        c = _iota((D, DP), 0)
        j = _iota((D, DP), 1)
        pm = jnp.logical_and(c == (j >> 5) * Dh + (j & 31), (j & 31) < Dh).astype(BF16)
        wv_s[...] = _dot(wqkv_ref[:, 2 * D:3 * D], pm).astype(BF16)
        kv_s[...] = jnp.zeros(kv_s.shape, F32)

    @pl.when(ph == 0)
    def _():
        x = x_ref[...].astype(F32)
        m = jnp.mean(x, axis=-1, keepdims=True)
        xc = x - m
        v = jnp.mean(xc * xc, axis=-1, keepdims=True)
        xn = (xc * jax.lax.rsqrt(v + 1e-5)).astype(BF16)

        pk = _dot(wqk_s[D:2 * D, :], xn, _NT)
        vp = _dot(xn, wv_s[...])
        lane = _iota(vp.shape, 1)
        vp = jnp.where((lane & 31) == Dh, 1.0, vp).astype(BF16)
        fk = _features(pk, Dh)
        for g in range(G):
            vg = vp[:, g * 128:(g + 1) * 128]
            kv_s[g, 0:R, :] += _dot(fk[g][0], vg)
            kv_s[g, R:2 * R, :] += _dot(fk[g][1], vg)
        pq = _dot(wqk_s[0:D, :], xn, _NT)
        fq = _features(pq, Dh)
        for g in range(G):
            phiq_s[t, g, 0:R, :] = fq[g][0]
            phiq_s[t, g, R:2 * R, :] = fq[g][1]

        @pl.when(t == 0)
        def _():
            cp1.wait()
            cp2.wait()

        acc = x + b2_ref[...].astype(F32)
        for c in range(F // FC):
            sl = slice(c * FC, (c + 1) * FC)
            h = _dot(xn, w1_s[:, sl]) + b1_ref[:, sl].astype(F32)
            h = jax.nn.gelu(h, approximate=True).astype(BF16)
            acc = acc + _dot(h, w2_s[sl, :])
        acc_s[t] = acc

    @pl.when(jnp.logical_and(ph == 1, t == 0))
    def _():
        cp3.wait()
        j = _iota((DP, D), 0)
        c = _iota((DP, D), 1)
        pmt = jnp.logical_and(c == (j >> 5) * Dh + (j & 31), (j & 31) < Dh).astype(BF16)
        wop_s[...] = _dot(pmt, wo_s[...]).astype(BF16)
        rr = _iota((256, 128), 0)
        cc = _iota((256, 128), 1)
        msk = (rr & 3) == (cc >> 5)
        for g in range(G):
            kvg = jnp.where(msk, kv_s[g], 0.0)
            kvt_s[g] = kvg.T[:, 0:2 * R].astype(BF16)

    @pl.when(ph == 1)
    def _():
        os_ = []
        for g in range(G):
            nd = _dot(kvt_s[g], phiq_s[t, g])
            for h4 in range(4):
                blk = nd[h4 * 32:(h4 + 1) * 32]
                den = blk[Dh:Dh + 1] + 1e-6
                os_.append((blk * (1.0 / den)).astype(BF16))
        ot = jnp.concatenate(os_, axis=0)
        o_ref[...] = (acc_s[t] + _dot(ot, wop_s[...], _TN)).astype(o_ref.dtype)


@jax.jit
def pallas_parallel_sum__linear_kernel_hedgehog__dense_activation_gelu__prompt_kernel(
    A_x, A_wqkv, A_w_phi, A_wo, B_x, B_w1, B_b1, B_w2, B_b2,
):
    import functools
    B, S, D = A_x.shape
    F = B_w1.shape[1]
    Dh = D // H
    assert B == 1 and S % TS == 0 and Dh < 32 and (4 * Dh) % 16 == 0
    nt = S // TS
    x = A_x.reshape(S, D)
    wphi = A_w_phi.reshape(D, Dh)
    b1 = B_b1.reshape(1, F)
    b2 = B_b2.reshape(1, D)
    const = lambda p, t: (0, 0)
    anyspec = pl.BlockSpec(memory_space=pl.ANY)
    out = pl.pallas_call(
        functools.partial(_kernel, D=D, F=F),
        grid=(2, nt),
        in_specs=[
            pl.BlockSpec((TS, D), lambda p, t: (t * (1 - p) + (nt - 1) * p, 0)),
            pl.BlockSpec((D, 3 * D), const),
            pl.BlockSpec((D, Dh), const),
            pl.BlockSpec((1, F), const),
            pl.BlockSpec((1, D), const),
            anyspec, anyspec, anyspec,
        ],
        out_specs=pl.BlockSpec((TS, D), lambda p, t: (t * p, 0)),
        out_shape=jax.ShapeDtypeStruct((S, D), A_x.dtype),
        scratch_shapes=[
            pltpu.VMEM((D, F), BF16),
            pltpu.VMEM((F, D), BF16),
            pltpu.VMEM((D, D), BF16),
            pltpu.VMEM((2 * D, D), BF16),
            pltpu.VMEM((D, H * 32), BF16),
            pltpu.VMEM((H * 32, D), BF16),
            pltpu.VMEM((G, 256, 128), F32),
            pltpu.VMEM((G, 128, 8 * Dh), BF16),
            pltpu.VMEM((nt, G, 8 * Dh, TS), BF16),
            pltpu.VMEM((nt, TS, D), F32),
            pltpu.SemaphoreType.DMA((3,)),
        ],
        compiler_params=pltpu.CompilerParams(
            dimension_semantics=("arbitrary", "arbitrary"),
            vmem_limit_bytes=100 * 1024 * 1024,
        ),
    )(x, A_wqkv, wphi, b1, b2, A_wo, B_w1, B_w2)
    return out.reshape(B, S, D)
```

```python
import jax
import jax.numpy as jnp
import jax.experimental.pallas as pl
import jax.experimental.pallas.tpu as pltpu

H = 16
G = 4
TS = 512
FC = 256

_NT = (((1,), (1,)), ((), ()))
_TN = (((0,), (0,)), ((), ()))
F32 = jnp.float32
BF16 = jnp.bfloat16


def _dot(a, b, dims=(((1,), (0,)), ((), ()))):
    return jax.lax.dot_general(a, b, dims, preferred_element_type=F32)


def _iota(shape, d):
    return jax.lax.broadcasted_iota(jnp.int32, shape, d)


def _fdiv(i, n):
    return jnp.floor((i.astype(F32) + 0.5) * (1.0 / n)).astype(jnp.int32)


def _features(p, Dh):
    T = p.shape[1]
    R = 4 * Dh
    n = R // 8
    outs = []
    for g in range(G):
        pg = p[g * R:(g + 1) * R].reshape(n, 8, T)
        mx = jnp.max(pg, axis=0)
        mn = jnp.min(pg, axis=0)
        mx = jnp.maximum(mx, pltpu.roll(mx, 4, 0))
        mn = jnp.minimum(mn, pltpu.roll(mn, 4, 0))
        e1 = jnp.exp(pg - mx[None])
        e2 = jnp.exp(mn[None] - pg)
        s1 = jnp.sum(e1, axis=0)
        s2 = jnp.sum(e2, axis=0)
        s1 = s1 + pltpu.roll(s1, 4, 0)
        s2 = s2 + pltpu.roll(s2, 4, 0)
        f1 = (e1 * (1.0 / s1)[None]).reshape(R, T).astype(BF16)
        f2 = (e2 * (1.0 / s2)[None]).reshape(R, T).astype(BF16)
        outs.append((f1, f2))
    return outs


def _kernel(x_ref, wqkv_ref, wphi_ref, b1_ref, b2_ref, wo_hbm, w1_hbm, w2_hbm,
            o_ref,
            w1_s, w1t_s, w2_s, wo_s, wqkv_s, wop_s, kv_s, kvt_s, phiq_s, acc_s, sems,
            *, D, F):
    ph = pl.program_id(0)
    t = pl.program_id(1)
    Dh = D // H
    R = 4 * Dh
    DP = H * 32

    cp1 = pltpu.make_async_copy(w1_hbm, w1_s.at[0:D], sems.at[0])
    cp2 = pltpu.make_async_copy(w2_hbm, w2_s, sems.at[1])
    cp3 = pltpu.make_async_copy(wo_hbm, wo_s, sems.at[2])

    @pl.when(jnp.logical_and(ph == 0, t == 0))
    def _():
        cp1.start()
        cp2.start()
        cp3.start()
        r = _iota((D, Dh), 0)
        f_r = (r - _fdiv(r, R) * R) >> 2
        et = (f_r == _iota((D, Dh), 1)).astype(BF16)
        r = _iota((D, D), 0)
        c = _iota((D, D), 1)
        head_r = _fdiv(r, R) * 4 + (r & 3)
        head_c = _fdiv(c, Dh)
        d_c = c - head_c * Dh
        sel = head_r == head_c
        bd = jnp.zeros((D, D), F32)
        eh = (_fdiv(_iota((D, H), 0), R) * 4 + (_iota((D, H), 0) & 3)
              == _iota((D, H), 1)).astype(BF16)
        for d in range(Dh):
            a = _dot(eh, wphi_ref[d])
            col = jnp.sum(a * et.astype(F32), axis=1, keepdims=True)
            bd = jnp.where(d_c == d, col, bd)
        bd = jnp.where(sel, bd, 0.0).astype(BF16)
        wqkv_s[0:D, :] = _dot(bd, wqkv_ref[:, 0:D], _NT).astype(BF16)
        wqkv_s[D:2 * D, :] = _dot(bd, wqkv_ref[:, D:2 * D], _NT).astype(BF16)
        j = _iota((DP, D), 0)
        c = _iota((DP, D), 1)
        pmt = jnp.logical_and(c == (j >> 5) * Dh + (j & 31), (j & 31) < Dh).astype(BF16)
        wqkv_s[2 * D:2 * D + DP, :] = _dot(pmt, wqkv_ref[:, 2 * D:3 * D], _NT).astype(BF16)
        kv_s[...] = jnp.zeros(kv_s.shape, F32)

    @pl.when(ph == 0)
    def _():
        x = x_ref[...].astype(F32)
        T = x.shape[1]
        m = jnp.mean(x, axis=0, keepdims=True)
        xc = x - m
        v = jnp.mean(xc * xc, axis=0, keepdims=True)
        xn = (xc * jax.lax.rsqrt(v + 1e-5)).astype(BF16)

        pk = _dot(wqkv_s[D:2 * D, :], xn)
        vp = _dot(wqkv_s[2 * D:2 * D + DP, :], xn)
        row = _iota(vp.shape, 0)
        vp = jnp.where((row & 31) == Dh, 1.0, vp).astype(BF16)
        fk = _features(pk, Dh)
        for g in range(G):
            vg = vp[g * 128:(g + 1) * 128]
            kv_s[g, 0:R, :] += _dot(fk[g][0], vg, _NT)
            kv_s[g, R:2 * R, :] += _dot(fk[g][1], vg, _NT)
        pq = _dot(wqkv_s[0:D, :], xn)
        fq = _features(pq, Dh)
        for g in range(G):
            phiq_s[t, g, 0:R, :] = fq[g][0]
            phiq_s[t, g, R:2 * R, :] = fq[g][1]

        @pl.when(t == 0)
        def _():
            cp1.wait()
            cp2.wait()
            rr = _iota((512 - D, F), 0)
            w1_s[D:512, :] = jnp.where(rr == 0, b1_ref[...].astype(F32), 0.0).astype(BF16)
            w1t_s[...] = w1_s[...].T

        aug = (_iota((512 - D, T), 0) == 0).astype(BF16)
        xa = jnp.concatenate([xn, aug], axis=0)
        acc = x
        for c in range(F // FC):
            sl = slice(c * FC, (c + 1) * FC)
            h = _dot(w1t_s[sl, :], xa)
            h = jax.nn.gelu(h, approximate=True).astype(BF16)
            acc = acc + _dot(w2_s[:, sl], h)
        acc_s[t] = acc

    @pl.when(jnp.logical_and(ph == 1, t == 0))
    def _():
        cp3.wait()
        j = _iota((DP, D), 0)
        c = _iota((DP, D), 1)
        pmt = jnp.logical_and(c == (j >> 5) * Dh + (j & 31), (j & 31) < Dh).astype(BF16)
        wop = _dot(pmt, wo_s[...])
        wop = jnp.where(j == Dh, b2_ref[...].astype(F32), wop)
        wop_s[...] = wop.T.astype(BF16)
        rr = _iota((256, 128), 0)
        cc = _iota((256, 128), 1)
        msk = (rr & 3) == (cc >> 5)
        for g in range(G):
            kvg = jnp.where(msk, kv_s[g], 0.0)
            kvt_s[g] = kvg.T[:, 0:2 * R].astype(BF16)

    @pl.when(ph == 1)
    def _():
        os_ = []
        for g in range(G):
            nd = _dot(kvt_s[g], phiq_s[t, g])
            for h4 in range(4):
                blk = nd[h4 * 32:(h4 + 1) * 32]
                den = blk[Dh:Dh + 1] + 1e-6
                o = blk * (1.0 / den)
                if g == 0 and h4 == 0:
                    o = jnp.where(_iota(o.shape, 0) == Dh, 1.0, o)
                os_.append(o.astype(BF16))
        ot = jnp.concatenate(os_, axis=0)
        o_ref[...] = (acc_s[t] + _dot(wop_s[...], ot)).astype(o_ref.dtype)


@jax.jit
def pallas_parallel_sum__linear_kernel_hedgehog__dense_activation_gelu__prompt_kernel(
    A_x, A_wqkv, A_w_phi, A_wo, B_x, B_w1, B_b1, B_w2, B_b2,
):
    import functools
    B, S, D = A_x.shape
    F = B_w1.shape[1]
    Dh = D // H
    assert B == 1 and S % TS == 0 and Dh < 32 and (4 * Dh) % 16 == 0 and D < 512
    nt = S // TS
    xt = A_x.reshape(S, D).T
    wphi = A_w_phi.transpose(1, 0, 2)
    b1 = B_b1.reshape(1, F)
    b2 = B_b2.reshape(1, D)
    const = lambda p, t: (0, 0)
    anyspec = pl.BlockSpec(memory_space=pl.ANY)
    out = pl.pallas_call(
        functools.partial(_kernel, D=D, F=F),
        grid=(2, nt),
        in_specs=[
            pl.BlockSpec((D, TS), lambda p, t: (0, t * (1 - p) + (nt - 1) * p)),
            pl.BlockSpec((D, 3 * D), const),
            pl.BlockSpec((Dh, H, Dh), lambda p, t: (0, 0, 0)),
            pl.BlockSpec((1, F), const),
            pl.BlockSpec((1, D), const),
            anyspec, anyspec, anyspec,
        ],
        out_specs=pl.BlockSpec((D, TS), lambda p, t: (0, t * p)),
        out_shape=jax.ShapeDtypeStruct((D, S), A_x.dtype),
        scratch_shapes=[
            pltpu.VMEM((512, F), BF16),
            pltpu.VMEM((F, 512), BF16),
            pltpu.VMEM((D, F), BF16),
            pltpu.VMEM((D, D), BF16),
            pltpu.VMEM((2 * D + H * 32, D), BF16),
            pltpu.VMEM((D, H * 32), BF16),
            pltpu.VMEM((G, 256, 128), F32),
            pltpu.VMEM((G, 128, 8 * Dh), BF16),
            pltpu.VMEM((nt, G, 8 * Dh, TS), BF16),
            pltpu.VMEM((nt, D, TS), F32),
            pltpu.SemaphoreType.DMA((3,)),
        ],
        compiler_params=pltpu.CompilerParams(
            dimension_semantics=("arbitrary", "arbitrary"),
            vmem_limit_bytes=100 * 1024 * 1024,
        ),
    )(xt, A_wqkv, wphi, b1, b2, A_wo, B_w1, B_w2.T)
    return out.T.reshape(B, S, D)
```

```python
import functools

import jax
import jax.numpy as jnp
import jax.experimental.pallas as pl
import jax.experimental.pallas.tpu as pltpu

H = 16
G = 4
TS = 1024
OC = 512
FC = 1792

_NT = (((1,), (1,)), ((), ()))
_TN = (((0,), (0,)), ((), ()))
F32 = jnp.float32
BF16 = jnp.bfloat16


def _dot(a, b, dims=(((1,), (0,)), ((), ()))):
    return jax.lax.dot_general(a, b, dims, preferred_element_type=F32)


def _iota(shape, d):
    return jax.lax.broadcasted_iota(jnp.int32, shape, d)


def _fdiv(i, n):
    return jnp.floor((i.astype(F32) + 0.5) * (1.0 / n)).astype(jnp.int32)


def _features(p, Dh):
    T = p.shape[1]
    R = 4 * Dh
    n = R // 8
    outs = []
    for g in range(G):
        pg = p[g * R:(g + 1) * R].reshape(n, 8, T)
        mx = jnp.max(pg, axis=0)
        mn = jnp.min(pg, axis=0)
        mx = jnp.maximum(mx, pltpu.roll(mx, 4, 0))
        mn = jnp.minimum(mn, pltpu.roll(mn, 4, 0))
        e1 = jnp.exp(pg - mx[None])
        e2 = jnp.exp(mn[None] - pg)
        s1 = jnp.sum(e1, axis=0)
        s2 = jnp.sum(e2, axis=0)
        s1 = s1 + pltpu.roll(s1, 4, 0)
        s2 = s2 + pltpu.roll(s2, 4, 0)
        f1 = (e1 * (1.0 / s1)[None]).reshape(R, T).astype(BF16)
        f2 = (e2 * (1.0 / s2)[None]).reshape(R, T).astype(BF16)
        outs.append((f1, f2))
    return outs


def _kernel(wphi_ref, b1_ref, b2_ref, x_hbm, wqkv_hbm, wo_hbm, w1_hbm, w2_hbm,
            o_hbm,
            x_s, wraw_s, w1_s, w2_s, wo_s, wqkv_s, kv_s, kvt_s, phiq_s, acc_s, out_s, sems, osems, wsems,
            *, D, F, nt):
    ph = pl.program_id(0)
    t = pl.program_id(1)
    Dh = D // H
    R = 4 * Dh

    wch = [(0, D)]
    cp0 = [pltpu.make_async_copy(wqkv_hbm.at[a:b], wraw_s.at[a:b], wsems.at[i])
           for i, (a, b) in enumerate(wch)]

    def xcp(i):
        return pltpu.make_async_copy(
            x_hbm.at[:, pl.ds(pl.multiple_of(i * TS, TS), TS)], x_s.at[i], sems.at[4 + i])

    cp1 = pltpu.make_async_copy(w1_hbm, w1_s.at[0:D], sems.at[0])
    cp2 = pltpu.make_async_copy(w2_hbm, w2_s, sems.at[1])
    cp3 = pltpu.make_async_copy(wo_hbm, wo_s.at[0:D], sems.at[2])

    @pl.when(jnp.logical_and(ph == 0, t == 0))
    def _():
        for cp in cp0:
            cp.start()
        r = _iota((D, D), 0)
        c = _iota((D, D), 1)
        head_rr = _fdiv(r, Dh)
        perm = (c == (r - head_rr * Dh) * H + head_rr).astype(BF16)
        wf = _dot(perm, wphi_ref[...]).astype(BF16)
        et = ((_iota((R, Dh), 0) >> 2) == _iota((R, Dh), 1)).astype(BF16)
        sel = (_iota((R, R), 0) & 3) == _fdiv(_iota((R, R), 1), Dh)
        eye = (_iota((R, R), 0) == _iota((R, R), 1)).astype(BF16)
        bds = [jnp.where(sel, _dot(et, wf[g * R:(g + 1) * R], _NT), 0.0).astype(BF16)
               for g in range(G)]
        for cp, (a, b) in zip(cp0, wch):
            cp.wait()
            xcp(0).start()
            cp1.start()
            cp2.start()
            for i in range(1, nt):
                xcp(i).start()
            cp3.start()
            for g in range(G):
                for i in range(3):
                    lo = i * D + g * R
                    lhs = bds[g] if i < 2 else eye
                    wqkv_s[lo:lo + R, a:b] = _dot(
                        lhs, wraw_s[a:b, lo:lo + R], _NT).astype(BF16)
        kv_s[...] = jnp.zeros(kv_s.shape, F32)

    @pl.when(ph == 0)
    def _():
        xcp(t).wait()
        x = x_s[t].astype(F32)
        T = x.shape[1]
        m = jnp.mean(x, axis=0, keepdims=True)
        xc = x - m
        v = jnp.mean(xc * xc, axis=0, keepdims=True)
        xn = (xc * jax.lax.rsqrt(v + 1e-5)).astype(BF16)

        pk = _dot(wqkv_s[D:2 * D, :], xn)
        vp = _dot(wqkv_s[2 * D:3 * D, :], xn).astype(BF16)
        ones4 = (_iota((128 - R, T), 0) < 4).astype(BF16)
        fk = _features(pk, Dh)
        for g in range(G):
            vg = jnp.concatenate([vp[g * R:(g + 1) * R], ones4], axis=0)
            kv_s[g, 0:R, :] += _dot(fk[g][0], vg, _NT)
            kv_s[g, R:2 * R, :] += _dot(fk[g][1], vg, _NT)
        pq = _dot(wqkv_s[0:D, :], xn)
        fq = _features(pq, Dh)
        for g in range(G):
            phiq_s[t, g, 0:R, :] = fq[g][0]
            phiq_s[t, g, R:2 * R, :] = fq[g][1]

        @pl.when(t == 0)
        def _():
            cp1.wait()
            cp2.wait()
            rr = _iota((512 - D, F), 0)
            w1_s[D:512, :] = jnp.where(rr == 0, b1_ref[...].astype(F32).reshape(1, F), 0.0).astype(BF16)

        aug = (_iota((512 - D, T), 0) == 0).astype(BF16)
        xa = jnp.concatenate([xn, aug], axis=0)
        acc = x
        for c in range(F // FC):
            sl = slice(c * FC, (c + 1) * FC)
            h = _dot(w1_s[:, sl], xa, _TN)
            h = jax.nn.gelu(h, approximate=True).astype(BF16)
            acc = acc + _dot(w2_s[:, sl], h)
        acc_s[t] = acc

    @pl.when(jnp.logical_and(ph == 1, t == 0))
    def _():
        cp3.wait()
        aux = jnp.where(_iota((512 - D, D), 0) == 0, b2_ref[...].astype(F32).reshape(1, D), 0.0)
        wo_s[D:512, :] = aux.astype(BF16)
        rr = _iota((256, 128), 0)
        cc = _iota((256, 128), 1)
        msk = (rr & 3) == jnp.where(cc < R, _fdiv(cc, Dh), cc - R)
        for g in range(G):
            kvg = jnp.where(msk, kv_s[g], 0.0)
            kvt_s[g] = kvg[0:2 * R].astype(BF16)

    def ocp(i):
        sl = pl.ds(pl.multiple_of(i * OC, OC), OC)
        return pltpu.make_async_copy(out_s.at[i], o_hbm.at[:, sl], osems.at[i])

    @pl.when(ph == 1)
    def _():
        nc = TS // OC
        for j in range(nc):
            cs = slice(j * OC, (j + 1) * OC)
            os_ = []
            hrow = _iota((R, OC), 0)
            for g in range(G):
                nd = _dot(kvt_s[g], phiq_s[t, g, :, cs], _TN)
                inv = 1.0 / (nd[R:R + 8] + 1e-6)
                den = inv[3:4]
                for h4 in (2, 1, 0):
                    den = jnp.where(hrow < (h4 + 1) * Dh, inv[h4:h4 + 1], den)
                os_.append((nd[0:R] * den).astype(BF16))
            os_.append((_iota((512 - D, OC), 0) == 0).astype(BF16))
            ot = jnp.concatenate(os_, axis=0)
            i = t * nc + j
            out_s[i] = (acc_s[t, :, cs] + _dot(wo_s[...], ot, _TN)).astype(out_s.dtype)
            ocp(i).start()

        @pl.when(t == nt - 1)
        def _():
            for i in range(nt * nc):
                ocp(i).wait()


@jax.jit
def pallas_parallel_sum__linear_kernel_hedgehog__dense_activation_gelu__prompt_kernel(
    A_x, A_wqkv, A_w_phi, A_wo, B_x, B_w1, B_b1, B_w2, B_b2,
):
    B, S, D = A_x.shape
    F = B_w1.shape[1]
    Dh = D // H
    assert B == 1 and S % TS == 0 and Dh < 32 and (4 * Dh) % 16 == 0 and D < 512
    nt = S // TS
    xt = A_x.reshape(S, D).T
    wphi = A_w_phi.transpose(1, 0, 2).reshape(D, Dh)
    const = lambda p, t: (0, 0)
    anyspec = pl.BlockSpec(memory_space=pl.ANY)
    out = pl.pallas_call(
        functools.partial(_kernel, D=D, F=F, nt=nt),
        grid=(2, nt),
        in_specs=[
            pl.BlockSpec((D, Dh), const),
            pl.BlockSpec((F,), lambda p, t: (0,)),
            pl.BlockSpec((D,), lambda p, t: (0,)),
            anyspec, anyspec, anyspec, anyspec, anyspec,
        ],
        out_specs=anyspec,
        out_shape=jax.ShapeDtypeStruct((D, S), A_x.dtype),
        scratch_shapes=[
            pltpu.VMEM((nt, D, TS), BF16),
            pltpu.VMEM((D, 3 * D), BF16),
            pltpu.VMEM((512, F), BF16),
            pltpu.VMEM((D, F), BF16),
            pltpu.VMEM((512, D), BF16),
            pltpu.VMEM((3 * D, D), BF16),
            pltpu.VMEM((G, 256, 128), F32),
            pltpu.VMEM((G, 8 * Dh, 128), BF16),
            pltpu.VMEM((nt, G, 8 * Dh, TS), BF16),
            pltpu.VMEM((nt, D, TS), F32),
            pltpu.VMEM((S // OC, D, OC), A_x.dtype),
            pltpu.SemaphoreType.DMA((4 + nt,)),
            pltpu.SemaphoreType.DMA((S // OC,)),
            pltpu.SemaphoreType.DMA((pl.cdiv(D, 128),)),
        ],
        compiler_params=pltpu.CompilerParams(
            dimension_semantics=("arbitrary", "arbitrary"),
            vmem_limit_bytes=100 * 1024 * 1024,
        ),
    )(wphi, B_b1, B_b2, xt, A_wqkv, A_wo, B_w1, B_w2.T)
    return out.T.reshape(B, S, D)
```
